```python
import os as _os
_os.environ.setdefault("JAX_PLATFORMS", "cpu")
import jax
import jax.numpy as jnp

def _softmax(x, axis=-1):
    return jax.nn.softmax(x, axis=axis)
def _gelu(x):
    return jax.nn.gelu(x, approximate=True)
def _silu(x):
    return jax.nn.silu(x)
def _sigmoid(x):
    return jax.nn.sigmoid(x)
def _layernorm(x, axis=-1, eps=1e-5):
    m = jnp.mean(x, axis=axis, keepdims=True)
    v = jnp.var(x, axis=axis, keepdims=True)
    return (x - m) / jnp.sqrt(v + eps)
def _scatter_add(tgt, idx, src, axis=0):
    return tgt.at[idx].add(src)
def _segment_sum(src, seg, n):
    return jax.ops.segment_sum(src, seg, n)
class _Rng:
    def __init__(self, key):
        self._k = key
    def _next(self):
        self._k, sub = jax.random.split(self._k)
        return sub
    def normal(self, shape):
        return jax.random.normal(self._next(), shape, dtype=jnp.bfloat16)
    def randint(self, lo, hi, shape):
        return jax.random.randint(self._next(), shape, lo, hi, dtype=jnp.int32)
    def uniform(self, shape, lo=0.0, hi=1.0):
        return jax.random.uniform(self._next(), shape, jnp.bfloat16, lo, hi)
    def permutation(self, n):
        return jax.random.permutation(self._next(), n)


kernel_name = 'parallel_sum__softmax_full_mha__swiglu_ffn__prompt'

def setup_inputs():
    _rng = _Rng(jax.random.key(int.from_bytes(__import__("os").urandom(4), "little")))
    _w = (lambda a: (lambda t: t.astype(jnp.bfloat16) if jnp.issubdtype(t.dtype, jnp.floating) else t)(jnp.asarray(a)))
    def _A_setup():
        B, S, D = 1, 2048, 640
        return {
            "x": _w((lambda *s: _rng.normal(s) * 0.05)(B, S, D)),
            "wqkv": _w((lambda *s: _rng.normal(s) * 0.1)(D, 3 * D)),
            "wo": _w((lambda *s: _rng.normal(s) * 0.05)(D, D)),
        }
    _A_in = _A_setup()

    def _B_setup():
        B, S, D, F = 1, 2048, 640, 1536
        return {
            "x": _w((lambda *s: _rng.normal(s) * 0.05)(B, S, D)),
            "w_gate": _w((lambda *s: _rng.normal(s) * 0.05)(D, F)),
            "w_up": _w((lambda *s: _rng.normal(s) * 0.05)(D, F)),
            "w_down": _w((lambda *s: _rng.normal(s) * 0.05)(F, D)),
        }
    _B_in = _B_setup()

    return {
        "A_x": _A_in["x"],
        "A_wqkv": _A_in["wqkv"],
        "A_wo": _A_in["wo"],
        "B_x": _B_in["x"],
        "B_w_gate": _B_in["w_gate"],
        "B_w_up": _B_in["w_up"],
        "B_w_down": _B_in["w_down"],
    }

def reference(A_x, A_wqkv, A_wo, B_x, B_w_gate, B_w_up, B_w_down):
    def _A_ref(x, wqkv, wo):
        B, S, D = x.shape
        H = 32; Dh = D // H
        qkv = (lambda x, *d: x.transpose(*d))((x @ wqkv).reshape(B, S, 3, H, Dh), 2, 0, 3, 1, 4)
        q, k, v = qkv[0], qkv[1], qkv[2]
        scale = Dh ** -0.5
        scores = jnp.einsum("bhqd,bhkd->bhqk", q, k) * scale
        p = _softmax(scores, axis=-1)
        o = jnp.einsum("bhqk,bhkd->bhqd", p, v)
        return (lambda x, *d: x.transpose(*d))(o, 0, 2, 1, 3).reshape(B, S, D) @ wo

    def _B_ref(x, w_gate, w_up, w_down):
        g = _silu(x @ w_gate)
        u = x @ w_up
        return (g * u) @ w_down

    x = A_x
    xn = _layernorm(x, axis=-1)
    return x + _A_ref(xn, A_wqkv, A_wo) + _B_ref(xn, B_w_gate, B_w_up, B_w_down)
```

```python
import math

import jax
import jax.numpy as jnp
from jax import lax
import jax.experimental.pallas as pl
import jax.experimental.pallas.tpu as pltpu

S, D, H, F = 2048, 640, 32, 1536
DH = D // H
NWIN = 9
RC = 512
OC = 256
TQ = 512
CK = 128
Q_SCALE = (DH ** -0.5) * math.log2(math.e)
F32, BF16 = jnp.float32, jnp.bfloat16


def _dot(a, b):
    return lax.dot_general(a, b, (((1,), (0,)), ((), ())), preferred_element_type=F32)


def _dot_nt(a, b):
    return lax.dot_general(a, b, (((1,), (1,)), ((), ())), preferred_element_type=F32)


def _kernel(x_hbm, wqkv_hbm, wo_hbm, wg_hbm, wu_hbm, wd_hbm, out_hbm,
            x_v, wqkv_v, wo_v, wg_v, wu_v, wd_v, xn_v, q_v, k_v, vt_v, vp_v,
            y_v, ot_v, sa_v, sb_v, m_v, out_v, x_sem, w_sem, o_sem):
    n_rc = S // RC
    x_cp = [pltpu.make_async_copy(x_hbm.at[pl.ds(r * RC, RC)], x_v.at[pl.ds(r * RC, RC)],
                                  x_sem.at[r]) for r in range(n_rc)]
    qkv_cp = [pltpu.make_async_copy(wqkv_hbm.at[:, pl.ds(i * D, D)], wqkv_v.at[i], w_sem.at[i])
              for i in range(3)]
    w_cp = [pltpu.make_async_copy(s, d, w_sem.at[3 + i]) for i, (s, d) in enumerate(
        [(wg_hbm, wg_v), (wu_hbm, wu_v), (wd_hbm, wd_v), (wo_hbm, wo_v)])]

    def layernorm(r):
        rows = pl.ds(r * RC, RC)
        x = x_v[rows, :].astype(F32)
        xc = x - jnp.mean(x, axis=-1, keepdims=True)
        var = jnp.mean(xc * xc, axis=-1, keepdims=True)
        xn_v[rows, :] = (xc * lax.rsqrt(var + 1e-5)).astype(BF16)

    for cp in [x_cp[0], qkv_cp[2], qkv_cp[0]]:
        cp.start()
    x_cp[0].wait()
    for cp in [qkv_cp[1], x_cp[1]]:
        cp.start()
    layernorm(0)
    for r in range(n_rc):
        rows = pl.ds(r * RC, RC)
        if r == 0:
            qkv_cp[2].wait()
        elif r + 1 < n_rc:
            x_cp[r + 1].wait()
            layernorm(r + 1)
        xn = xn_v[rows, :]
        vt_v[:, rows] = _dot(xn, wqkv_v[2]).T
        if r == 0:
            for cp in [qkv_cp[0], qkv_cp[1], x_cp[1]]:
                cp.wait()
            for cp in x_cp[2:]:
                cp.start()
            layernorm(1)
        if r == 1:
            for cp in w_cp:
                cp.start()
        q = _dot(xn, wqkv_v[0]) * Q_SCALE
        k = _dot(xn, wqkv_v[1])
        for val, ref in ((q, q_v), (k, k_v)):
            for w in range(NWIN):
                lo = 128 * w if w < 5 else 128 * (w - 5) + 64
                ref[w, rows, :] = val[:, lo:lo + 128].astype(BF16)

    def build_v_heads():
        row8 = lax.broadcasted_iota(jnp.int32, (8, S), 0)
        for h in range(H):
            st = (DH * h) // 8 * 8
            g = [vt_v[pl.ds(st + 8 * i, 8), :] for i in range(3)]
            if h % 2 == 0:
                g[2] = jnp.where(row8 >= 4, 1.0, g[2])
            else:
                g[0] = jnp.where(row8 < 4, 1.0, g[0])
            for i in range(3):
                vp_v[h, pl.ds(8 * i, 8), :] = g[i]

    for cp in w_cp:
        cp.wait()

    def ffn(r, carry):
        rows = pl.ds(pl.multiple_of(r * RC, RC), RC)
        xn = xn_v[rows, :]
        acc = x_v[rows, :].astype(F32)
        for c in range(F // 512):
            cols = pl.ds(c * 512, 512)
            g = _dot(xn, wg_v[:, cols])
            u = _dot(xn, wu_v[:, cols])
            a = (g / (1.0 + jnp.exp(-g)) * u).astype(BF16)
            acc = acc + _dot(a, wd_v[cols, :])
        y_v[rows, :] = acc
        return carry

    lax.fori_loop(0, n_rc, ffn, None)

    lane = lax.broadcasted_iota(jnp.int32, (TQ, 128), 1)
    row8q = lax.broadcasted_iota(jnp.int32, (8, TQ), 0)

    def window(h):
        start = h * DH
        c = start // 128
        off = start - 128 * c
        cross = off + DH > 128
        return jnp.where(cross, c + 5, c), jnp.where(cross, off - 64, off)

    def step(h, odd, cur, nxt, do_qk, do_pv, after_tile=None):
        if do_qk:
            w, off = window(h + 1)
        for qb in range(S // TQ):
            qs = pl.ds(qb * TQ, TQ)
            if do_qk:
                qm = q_v[w, qs, :]
                qm = jnp.where((lane >= off) & (lane < off + DH), qm, jnp.zeros_like(qm))
            if do_pv:
                m = m_v[odd, :, qs]
            acc = mx = None
            for c in range(S // CK):
                ks = pl.ds(c * CK, CK)
                if do_pv:
                    p = jnp.exp2(cur[ks, qs] - m).astype(BF16)
                    a = _dot(vp_v[h, :, ks], p)
                    acc = a if acc is None else acc + a
                if do_qk:
                    s = _dot_nt(k_v[w, ks, :], qm)
                    nxt[ks, qs] = s
                    t = jnp.max(s.reshape(CK // 8, 8, TQ), axis=0)
                    mx = t if mx is None else jnp.maximum(mx, t)
            if do_qk:
                m_v[1 - odd, :, qs] = jnp.max(mx, axis=0, keepdims=True)
            if do_pv:
                o = acc * (1.0 / (acc[0:1] if odd else acc[23:24]))
                st = pl.multiple_of((h // 2) * 40 + (16 if odd else 0), 8)
                if odd:
                    old = ot_v[pl.ds(st, 8), qs]
                    ot_v[pl.ds(st, 8), qs] = jnp.where(row8q < 4, old, o[0:8])
                    ot_v[pl.ds(st + 8, 16), qs] = o[8:24]
                else:
                    ot_v[pl.ds(st, 24), qs] = o
            if after_tile is not None:
                after_tile(qb)

    step(-1, 1, None, sa_v, True, False)
    build_v_heads()

    def head(i, carry):
        step(2 * i, 0, sa_v, sb_v, True, True)
        step(2 * i + 1, 1, sb_v, sa_v, True, True)
        return carry

    lax.fori_loop(0, H // 2 - 1, head, None)
    step(H - 2, 0, sa_v, sb_v, True, True)

    o_cp = [pltpu.make_async_copy(out_v.at[pl.ds(r * OC, OC)], out_hbm.at[pl.ds(r * OC, OC)],
                                  o_sem.at[r]) for r in range(S // OC)]

    def project(qb):
        for r in range(qb * TQ // OC, (qb + 1) * TQ // OC):
            rows = pl.ds(r * OC, OC)
            o = ot_v[:, rows].T.astype(BF16)
            out_v[rows, :] = (y_v[rows, :] + _dot(o, wo_v[...])).astype(BF16)

    step(H - 1, 1, sb_v, None, False, True, lambda qb: project(qb - 1) if qb else None)
    half = len(o_cp) - TQ // OC
    for cp in o_cp[:half]:
        cp.start()
    project(S // TQ - 1)
    for cp in o_cp[half:]:
        cp.start()
    for cp in o_cp:
        cp.wait()


@jax.jit
def pallas_parallel_sum__softmax_full_mha__swiglu_ffn__prompt_kernel(
    A_x: jax.Array,
    A_wqkv: jax.Array,
    A_wo: jax.Array,
    B_x: jax.Array,
    B_w_gate: jax.Array,
    B_w_up: jax.Array,
    B_w_down: jax.Array,
):
    del B_x
    vm = pltpu.VMEM
    out = pl.pallas_call(
        _kernel,
        out_shape=jax.ShapeDtypeStruct((S, D), BF16),
        in_specs=[pl.BlockSpec(memory_space=pl.ANY)] * 6,
        out_specs=pl.BlockSpec(memory_space=pl.ANY),
        scratch_shapes=[
            vm((S, D), BF16), vm((3, D, D), BF16), vm((D, D), BF16),
            vm((D, F), BF16), vm((D, F), BF16), vm((F, D), BF16),
            vm((S, D), BF16), vm((NWIN, S, 128), BF16), vm((NWIN, S, 128), BF16),
            vm((D, S), F32), vm((H, 24, S), F32),
            vm((S, D), F32), vm((D, S), F32), vm((S, S), F32), vm((S, S), F32),
            vm((2, 1, S), F32), vm((S, D), BF16),
            pltpu.SemaphoreType.DMA((S // RC,)), pltpu.SemaphoreType.DMA((7,)),
            pltpu.SemaphoreType.DMA((S // OC,)),
        ],
        compiler_params=pltpu.CompilerParams(vmem_limit_bytes=110 * 2 ** 20),
        name="fused_block",
    )(A_x.reshape(S, D), A_wqkv, A_wo, B_w_gate, B_w_up, B_w_down)
    return out.reshape(1, S, D)
```
